```python
import os as _os
_os.environ.setdefault("JAX_PLATFORMS", "cpu")
import jax
import jax.numpy as jnp

def _softmax(x, axis=-1):
    return jax.nn.softmax(x, axis=axis)
def _gelu(x):
    return jax.nn.gelu(x, approximate=True)
def _silu(x):
    return jax.nn.silu(x)
def _sigmoid(x):
    return jax.nn.sigmoid(x)
def _layernorm(x, axis=-1, eps=1e-5):
    m = jnp.mean(x, axis=axis, keepdims=True)
    v = jnp.var(x, axis=axis, keepdims=True)
    return (x - m) / jnp.sqrt(v + eps)
def _scatter_add(tgt, idx, src, axis=0):
    return tgt.at[idx].add(src)
def _segment_sum(src, seg, n):
    return jax.ops.segment_sum(src, seg, n)
class _Rng:
    def __init__(self, key):
        self._k = key
    def _next(self):
        self._k, sub = jax.random.split(self._k)
        return sub
    def normal(self, shape):
        return jax.random.normal(self._next(), shape, dtype=jnp.bfloat16)
    def randint(self, lo, hi, shape):
        return jax.random.randint(self._next(), shape, lo, hi, dtype=jnp.int32)
    def uniform(self, shape, lo=0.0, hi=1.0):
        return jax.random.uniform(self._next(), shape, jnp.bfloat16, lo, hi)
    def permutation(self, n):
        return jax.random.permutation(self._next(), n)


kernel_name = 'concat_heads__gqa_block_cached__sliding_block_cached__decode'

def setup_inputs():
    _rng = _Rng(jax.random.key(int.from_bytes(__import__("os").urandom(4), "little")))
    _w = (lambda a: (lambda t: t.astype(jnp.bfloat16) if jnp.issubdtype(t.dtype, jnp.floating) else t)(jnp.asarray(a)))
    def _A_setup():
        B, Sq, D = 1, 1, 576
        Hq, Hkv, Sk, Dh = 32, 16, 8192, 128
        assert Hq % Hkv == 0, (Hq, Hkv)
        return {
            "x": _w((lambda *s: _rng.normal(s) * 0.8)(B, Sq, D)),
            "k_cache": _w((lambda *s: _rng.normal(s) * 0.8)(B, Hkv, Sk, Dh)),
            "v_cache": _w((lambda *s: _rng.normal(s) * 0.05)(B, Hkv, Sk, Dh)),
            "wq": _w((lambda *s: _rng.normal(s) * 0.8)(D, Hq * Dh) * (D ** -0.5)),
            "wo": _w((lambda *s: _rng.normal(s) * 0.05)(Hq * Dh, D) * ((Hq * Dh) ** -0.5)),
        }
    _A_in = _A_setup()

    def _B_setup():
        B, Sq, D = 1, 1, 576
        Hq, Hkv, Sk, Dh = 32, 16, 8192, 128
        assert Hq % Hkv == 0, (Hq, Hkv)
        return {
            "x": _w((lambda *s: _rng.normal(s) * 0.8)(B, Sq, D)),
            "k_cache": _w((lambda *s: _rng.normal(s) * 0.8)(B, Hkv, Sk, Dh)),
            "v_cache": _w((lambda *s: _rng.normal(s) * 0.05)(B, Hkv, Sk, Dh)),
            "wq": _w((lambda *s: _rng.normal(s) * 0.8)(D, Hq * Dh) * (D ** -0.5)),
            "wo": _w((lambda *s: _rng.normal(s) * 0.05)(Hq * Dh, D) * ((Hq * Dh) ** -0.5)),
        }
    _B_in = _B_setup()

    return {
        "A_x": _A_in["x"],
        "A_k_cache": _A_in["k_cache"],
        "A_v_cache": _A_in["v_cache"],
        "A_wq": _A_in["wq"],
        "A_wo": _A_in["wo"],
        "B_x": _B_in["x"],
        "B_k_cache": _B_in["k_cache"],
        "B_v_cache": _B_in["v_cache"],
        "B_wq": _B_in["wq"],
        "B_wo": _B_in["wo"],
    }

def reference(A_x, A_k_cache, A_v_cache, A_wq, A_wo, B_x, B_k_cache, B_v_cache, B_wq, B_wo):
    def _A_ref(x, k_cache, v_cache, wq, wo):
        B, Sq, D = x.shape
        Hq, Dh = 32, 128
        Hkv = k_cache.shape[1]
        rep = Hq // Hkv
        q = (lambda x, *d: x.transpose(*d))((x @ wq).reshape(B, Sq, Hq, Dh), 0, 2, 1, 3)
        k = jnp.repeat(k_cache, rep, axis=1)
        v = jnp.repeat(v_cache, rep, axis=1)
        scores = jnp.einsum("bhqd,bhkd->bhqk", q, k) * (Dh ** -0.5)
        p = _softmax(scores, axis=-1)
        o = jnp.einsum("bhqk,bhkd->bhqd", p, v)
        return (lambda x, *d: x.transpose(*d))(o, 0, 2, 1, 3).reshape(B, Sq, Hq * Dh) @ wo

    def _B_ref(x, k_cache, v_cache, wq, wo):
        B, Sq, D = x.shape
        Hq, Dh = 32, 128
        Hkv, Sk = k_cache.shape[1], k_cache.shape[2]
        W = min(4096, max(256, Sk // 4))
        rep = Hq // Hkv
        q = (lambda x, *d: x.transpose(*d))((x @ wq).reshape(B, Sq, Hq, Dh), 0, 2, 1, 3)
        k = jnp.repeat(k_cache[:, :, Sk - W:, :], rep, axis=1)
        v = jnp.repeat(v_cache[:, :, Sk - W:, :], rep, axis=1)
        scores = jnp.einsum("bhqd,bhkd->bhqk", q, k) * (Dh ** -0.5)
        p = _softmax(scores, axis=-1)
        o = jnp.einsum("bhqk,bhkd->bhqd", p, v)
        return (lambda x, *d: x.transpose(*d))(o, 0, 2, 1, 3).reshape(B, Sq, Hq * Dh) @ wo

    a = _A_ref(A_x, A_k_cache, A_v_cache, A_wq, A_wo)
    b = _B_ref(B_x, B_k_cache, B_v_cache, B_wq, B_wo)
    return jnp.concatenate([a, b], axis=-1)
```

```python
import functools

import jax
import jax.numpy as jnp
from jax import lax
import jax.experimental.pallas as pl
import jax.experimental.pallas.tpu as pltpu

D, HQ, HKV, SK, DH = 576, 32, 16, 8192, 128
WIN = 2048
NT = (((1,), (1,)), ((), ()))
bf16, f32 = jnp.bfloat16, jnp.float32


def make(L=3, compute=True, dma=True, nosem=True, nobounds=True, nsem=8):
    NW, NA, NB, NO = 8, 64, 16, 8
    A0, B0, O0, END = NW, NW + NA, NW + NA + NB, NW + NA + NB + NO

    def kernel(xa, ka, va, wqa, woa, xb, kb, vb, wqb, wob, out,
               xbuf, wqbuf, wobuf, kvbuf, qbuf, mbuf, lbuf, accbuf, obuf, ybuf,
               sems, wsem, xsem):
        def sem(s):
            return sems.at[lax.rem(s, nsem)]

        def start_wq(i):
            r = pl.multiple_of(i * 8, 8)

            def body(j, _):
                c = pl.multiple_of(j * 512, 512)
                for s in range(3):
                    for a, w in enumerate((wqa, wqb)):
                        idx = (pl.ds(3 * s, 3), pl.ds(r, 8), pl.ds(c, 512))
                        pltpu.make_async_copy(w.at[idx], wqbuf.at[(a,) + idx], wsem).start(priority=a)
            lax.fori_loop(0, 8, body, None)

        def start_a(g):
            h0 = (g // 16) * 4
            t = lax.rem(g, 16) * 128

            def body(r, _):
                row = pl.multiple_of(t + r * 32, 32)
                for i in range(4):
                    for a, c in enumerate((ka, va)):
                        pltpu.make_async_copy(c.at[h0 + i, :, pl.ds(row, 32)],
                                              kvbuf.at[g, a, i, pl.ds(r * 4, 4)], sem(g)).start(priority=a)
            lax.fori_loop(0, 4, body, None)

        def start_b(g):
            gb = g - NA
            h0 = (gb // 4) * 4
            t = lax.rem(gb, 4) * 512

            def body(r4, _):
                for i in range(4):
                    r = r4 * 4 + i
                    row = pl.multiple_of(t + r * 32, 32)
                    for a, c in enumerate((kb, vb)):
                        pltpu.make_async_copy(c.at[pl.ds(h0, 4), 3, pl.ds(row, 32)],
                                              kvbuf.at[g, a, :, r], sem(g)).start(priority=a)
            lax.fori_loop(0, 4, body, None)

        def start_wo(j):
            c = pl.multiple_of(j * 512, 512)

            def body(i, _):
                r = pl.multiple_of(i * 8, 8)
                for s in range(3):
                    for a, w in enumerate((woa, wob)):
                        pltpu.make_async_copy(w.at[pl.ds(3 * s, 3), pl.ds(r, 8), pl.ds(c, 512)],
                                              wobuf.at[j, pl.ds(9 * a + 3 * s, 3), pl.ds(r, 8)],
                                              sem(NA + NB + j)).start(priority=a)
            lax.fori_loop(0, 8, body, None)

        def wait(ref, s):
            if dma:
                pltpu.make_async_copy(ref, ref, s).wait()

        row = lax.broadcasted_iota(jnp.int32, (8, 128), 0)

        def attend(g):
            is_b = g >= NA
            gb = g - NA
            a = is_b.astype(jnp.int32)
            blk = jnp.where(is_b, gb // 4, g // 16)
            first = jnp.where(is_b, lax.rem(gb, 4) == 0, lax.rem(g, 16) == 0)
            last = jnp.where(is_b, lax.rem(gb, 4) == 3, lax.rem(g, 16) == 15)
            col = pl.multiple_of(blk * 1024, 1024)

            @pl.when(first)
            def _():
                x = jnp.broadcast_to(xbuf[a].astype(f32), (8, D)).astype(bf16)
                w = wqbuf[a, :, :, pl.ds(col, 1024)].reshape(D, 1024)
                q = jnp.dot(x, w, preferred_element_type=f32)
                qb = q[:, :128]
                for r in range(1, 8):
                    qb = jnp.where(row == r, q[:, 128 * r:128 * (r + 1)], qb)
                qbuf[...] = qb
                mbuf[...] = jnp.full((8, 128), -jnp.inf, f32)
                lbuf[...] = jnp.zeros((8, 128), f32)
                accbuf[...] = jnp.zeros((8, 128), f32)

            q = qbuf[...].astype(bf16)
            row4 = lax.broadcasted_iota(jnp.int32, (8, 512), 0)
            s = None
            for i in range(4):
                k = kvbuf[g, 0, i].reshape(512, DH)
                si = lax.dot_general(q, k, NT, preferred_element_type=f32)
                s = si if i == 0 else jnp.where(row4 >= 2 * i, si, s)
            s = s * (DH ** -0.5)
            m_old = mbuf[...]
            m_new = jnp.maximum(m_old, jnp.max(s, axis=1, keepdims=True))
            alpha = jnp.exp(m_old - m_new)
            p = jnp.exp(s - jnp.concatenate([m_new] * 4, axis=1))
            l_new = alpha * lbuf[...] + (p[:, :128] + p[:, 128:256] + p[:, 256:384] + p[:, 384:])
            pb = p.astype(bf16)
            pv = None
            for i in range(4):
                v = kvbuf[g, 1, i].reshape(512, DH)
                oi = jnp.dot(pb, v, preferred_element_type=f32)
                pv = oi if i == 0 else jnp.where(row >= 2 * i, oi, pv)
            acc = alpha * accbuf[...] + pv
            mbuf[...] = m_new
            lbuf[...] = l_new
            accbuf[...] = acc

            @pl.when(last)
            def _():
                o = acc / jnp.sum(l_new, axis=1, keepdims=True)
                obuf[a, :, pl.ds(col, 1024)] = jnp.concatenate(
                    [jnp.broadcast_to(o[r:r + 1], (8, 128)) for r in range(8)], axis=1)

        def project(j):
            c = pl.multiple_of(j * 512, 512)
            row4 = lax.broadcasted_iota(jnp.int32, (8, 512), 0)
            o = jnp.where(row4 < 4, obuf[0, :, pl.ds(c, 512)], obuf[1, :, pl.ds(c, 512)]).astype(bf16)
            w = wobuf[j].reshape(2 * D, 512)
            y = lax.dot_general(o, w, NT, preferred_element_type=f32)
            ybuf[...] += y

        if dma:
            start_wq(0)
            cxa = pltpu.make_async_copy(xa.at[0], xbuf.at[0], xsem)
            cxb = pltpu.make_async_copy(xb.at[0], xbuf.at[1], xsem)
            cxa.start()
            cxb.start(priority=1)
        ybuf[...] = jnp.zeros(ybuf.shape, f32)

        def step(s, _):
            if dma:
                pl.when(s < A0)(lambda: start_wq(s))
                pl.when((s >= A0) & (s < B0))(lambda: start_a(s - A0))
                pl.when((s >= B0) & (s < O0))(lambda: start_b(s - A0))
                pl.when((s >= O0) & (s < END))(lambda: start_wo(s - O0))
            t = s - L

            @pl.when(t == A0)
            def _():
                wait(xbuf, xsem)
                wait(wqbuf, wsem)

            @pl.when((t >= A0) & (t < O0))
            def _():
                wait(kvbuf.at[0], sem(t - A0))
                if compute:
                    attend(t - A0)

            @pl.when(t >= O0)
            def _():
                wait(wobuf.at[0], sem(t - A0))
                if compute:
                    project(t - O0)

        lax.fori_loop(1, END + L, step, None)
        y = ybuf[...]
        lane = lax.broadcasted_iota(jnp.int32, (1, 2 * D), 1)
        out[0] = jnp.where(lane < D, y[0:1], y[4:5]).astype(bf16)

    def f(xa, ka, va, wqa, woa, xb, kb, vb, wqb, wob):
        kv = lambda c: c.reshape(HKV, SK // WIN, WIN, DH)
        w = lambda m: m.reshape(9, 64, HQ * DH)
        return pl.pallas_call(
            kernel,
            out_shape=jax.ShapeDtypeStruct((1, 1, 2 * D), bf16),
            in_specs=[pl.BlockSpec(memory_space=pltpu.HBM)] * 10,
            scratch_shapes=[
                pltpu.VMEM((2, 1, D), bf16),
                pltpu.VMEM((2, 9, 64, HQ * DH), bf16),
                pltpu.VMEM((8, 18, 64, 512), bf16),
                pltpu.VMEM((NA + NB, 2, 4, 16, 32, DH), bf16),
                pltpu.VMEM((8, 128), f32),
                pltpu.VMEM((8, 128), f32),
                pltpu.VMEM((8, 128), f32),
                pltpu.VMEM((8, 128), f32),
                pltpu.VMEM((2, 8, HQ * DH), f32),
                pltpu.VMEM((8, 2 * D), f32),
                pltpu.SemaphoreType.DMA((nsem,)),
                pltpu.SemaphoreType.DMA(()),
                pltpu.SemaphoreType.DMA(()),
            ],
            compiler_params=pltpu.CompilerParams(
                vmem_limit_bytes=120 * 2**20, disable_bounds_checks=nobounds,
                disable_semaphore_checks=nosem),
        )(xa, kv(ka), kv(va), w(wqa), w(woa.T), xb, kv(kb), kv(vb), w(wqb), w(wob.T))
    return f


@jax.jit
def pallas_concat_heads__gqa_block_cached__sliding_block_cached__decode_kernel(
    A_x, A_k_cache, A_v_cache, A_wq, A_wo, B_x, B_k_cache, B_v_cache, B_wq, B_wo
):
    return make()(A_x, A_k_cache, A_v_cache, A_wq, A_wo, B_x, B_k_cache, B_v_cache, B_wq, B_wo)
```

```python
import functools

import jax
import jax.numpy as jnp
import numpy as np
from jax import lax
import jax.experimental.pallas as pl
import jax.experimental.pallas.tpu as pltpu

D, HQ, HKV, SK, DH = 576, 32, 16, 8192, 128
WINDOW = min(4096, max(256, SK // 4))

SLAB = 64
NSLAB = D // SLAB

HEADS, KEYS, PIECE = 4, 512, 64
BLOCK_COLS = 2 * HEADS * DH
B_STEPS, A_STEPS = WINDOW // KEYS, SK // KEYS
B_GROUPS = B_STEPS * HKV // HEADS
GROUPS = B_GROUPS + A_STEPS * HKV // HEADS

LAG = 3

TAIL_COL = HQ * DH - BLOCK_COLS
TAIL = (
    ((((0, 2), (6, 2)), ((2, 2), (10, 2))), (0, 6)),
    ((((8, 1), (12, 2)), ((9, 1), (14, 2))), (6, 2)),
    ((((4, 2), (16, 2)),), (8, 1)),
)

NT_DIMS = (((1,), (1,)), ((), ()))
LOWEST = float(np.finfo(np.float32).min)


def _body(xa, ka, va, wqa, woa, xb, kb, vb, wqb, wob, out_ref,
          x_buf, wq_buf, wo_buf, kv_buf, q_ref, m_ref, l_ref, acc_ref, o_ref, y_ref,
          x_sem, wq_sem, wo_sem, kv_sems, tail_sems):
    f32, bf16 = jnp.float32, jnp.bfloat16

    def wait_for(buf, sem):
        pltpu.make_async_copy(buf, buf, sem).wait()

    def start_weights(srcs, dst, ncols, sem):
        @pl.loop(0, SLAB // 8)
        def _(i):
            rows = pl.ds(pl.multiple_of(i * 8, 8), 8)

            @pl.loop(0, ncols // 512)
            def _(j):
                cols = pl.ds(pl.multiple_of(j * 512, 512), 512)
                for s in range(0, NSLAB, 3):
                    for side, src in enumerate(srcs):
                        pltpu.make_async_copy(
                            src.at[pl.ds(s, 3), rows, cols],
                            dst.at[pl.ds(side * NSLAB + s, 3), rows, cols],
                            sem).start(priority=side)

    def start_b(g, sem):
        head = lax.div(g, B_STEPS) * HEADS
        key = SK // 2 - WINDOW + lax.rem(g, B_STEPS) * KEYS

        @pl.loop(0, KEYS // PIECE)
        def _(r):
            rows = pl.ds(pl.multiple_of(key + r * PIECE, PIECE), PIECE)
            for h in range(0, HEADS, 2):
                for c, cache in enumerate((kb, vb)):
                    pltpu.make_async_copy(
                        cache.at[pl.ds(head + h, 2), 1, rows],
                        kv_buf.at[g, c, pl.ds(h, 2), r], sem).start(priority=c)

    def start_a(g, sem):
        head = lax.div(g - B_GROUPS, A_STEPS) * HEADS
        key = lax.rem(g - B_GROUPS, A_STEPS) * (KEYS // 2)

        @pl.loop(0, KEYS // PIECE // 2)
        def _(r):
            rows = pl.ds(pl.multiple_of(key + r * PIECE, PIECE), PIECE)
            for h in range(HEADS):
                for c, cache in enumerate((ka, va)):
                    pltpu.make_async_copy(
                        cache.at[head + h, :, rows],
                        kv_buf.at[g, c, h, pl.ds(2 * r, 2)], sem).start(priority=c)

    def start_tail(k):
        cols = pl.ds(TAIL_COL, BLOCK_COLS)

        @pl.loop(0, SLAB // 8)
        def _(i):
            rows = pl.ds(pl.multiple_of(i * 8, 8), 8)
            for pair in TAIL[k][0]:
                for queue, (s, n) in enumerate(pair):
                    pltpu.make_async_copy(
                        (woa, wob)[s // NSLAB].at[pl.ds(s % NSLAB, n), rows, cols],
                        wo_buf.at[pl.ds(s, n), rows, cols],
                        tail_sems.at[k * queue]).start(priority=queue)

    def attend(g):
        is_b = g < B_GROUPS
        side = is_b.astype(jnp.int32)
        block = jnp.where(is_b, lax.div(g, B_STEPS), lax.div(g - B_GROUPS, A_STEPS))
        pos = jnp.where(is_b, lax.rem(g, B_STEPS), lax.rem(g - B_GROUPS, A_STEPS))
        cols = pl.ds(pl.multiple_of(block * BLOCK_COLS, BLOCK_COLS), BLOCK_COLS)
        row = lax.broadcasted_iota(jnp.int32, (8, DH), 0)

        @pl.when(pos == 0)
        def _():
            x = jnp.broadcast_to(x_buf[side].astype(f32), (8, D)).astype(bf16)
            wq = wq_buf[pl.ds(side * NSLAB, NSLAB), :, cols].reshape(D, BLOCK_COLS)
            q_all = jnp.dot(x, wq, preferred_element_type=f32)
            q = q_all[:, :DH]
            for r in range(1, 8):
                q = jnp.where(row == r, q_all[:, r * DH:(r + 1) * DH], q)
            q_ref[...] = q
            m_ref[...] = jnp.full((8, DH), LOWEST, f32)
            l_ref[...] = jnp.zeros((8, DH), f32)
            acc_ref[...] = jnp.zeros((8, DH), f32)

        def per_head(fn, width):
            r = lax.broadcasted_iota(jnp.int32, (8, width), 0)
            res = fn(0)
            for h in range(1, HEADS):
                res = jnp.where(r >= 2 * h, fn(h), res)
            return res

        q = q_ref[...].astype(bf16)
        s = per_head(lambda h: lax.dot_general(
            q, kv_buf[g, 0, h].reshape(KEYS, DH), NT_DIMS, preferred_element_type=f32), KEYS)
        s = s * (DH ** -0.5)
        m_old = m_ref[...]
        m_new = jnp.maximum(m_old, jnp.max(s, axis=1, keepdims=True))
        alpha = jnp.exp(m_old - m_new)
        p = jnp.exp(s - jnp.concatenate([m_new] * (KEYS // DH), axis=1))
        l_new = alpha * l_ref[...]
        for c in range(0, KEYS, DH):
            l_new += p[:, c:c + DH]
        p = p.astype(bf16)
        acc = alpha * acc_ref[...] + per_head(lambda h: jnp.dot(
            p, kv_buf[g, 1, h].reshape(KEYS, DH), preferred_element_type=f32), DH)
        m_ref[...] = m_new
        l_ref[...] = l_new
        acc_ref[...] = acc

        @pl.when(pos == jnp.where(is_b, B_STEPS - 1, A_STEPS - 1))
        def _():
            o = acc / jnp.sum(l_new, axis=1, keepdims=True)
            o_ref[side, :, cols] = jnp.concatenate(
                [jnp.broadcast_to(o[r:r + 1], (8, DH)) for r in range(8)], axis=1)

    def attention_out(cols):
        r = lax.broadcasted_iota(jnp.int32, (8, cols.size), 0)
        return jnp.where(r < 4, o_ref[0, :, cols], o_ref[1, :, cols]).astype(bf16)

    def project(j):
        cols = pl.ds(pl.multiple_of(j * 512, 512), 512)
        y_ref[...] += lax.dot_general(
            attention_out(cols), wo_buf[:, :, cols].reshape(2 * D, 512), NT_DIMS,
            preferred_element_type=f32)

    start_weights((wqa, wqb), wq_buf, HQ * DH, wq_sem)
    for side, x in enumerate((xa, xb)):
        pltpu.make_async_copy(x.at[0], x_buf.at[side], x_sem).start(priority=side)
    y_ref[...] = jnp.zeros(y_ref.shape, f32)
    start_weights((woa, wob), wo_buf, TAIL_COL, wo_sem)
    wait_for(wq_buf, wq_sem)
    wait_for(x_buf, x_sem)

    @pl.loop(0, GROUPS + LAG)
    def _(step):
        sem = kv_sems.at[lax.rem(step, LAG + 1)]
        pl.when(step < B_GROUPS)(lambda: start_b(step, sem))
        pl.when((step >= B_GROUPS) & (step < GROUPS))(lambda: start_a(step, sem))
        for k in range(len(TAIL)):
            pl.when(step == GROUPS + k)(lambda k=k: start_tail(k))

        g = step - LAG

        @pl.when(g >= 0)
        def _():
            wait_for(kv_buf.at[g], kv_sems.at[lax.rem(g, LAG + 1)])
            attend(g)

        j = g - (GROUPS - A_STEPS + 1)
        pl.when(j == 0)(lambda: wait_for(wo_buf.at[:, :, pl.ds(0, TAIL_COL)], wo_sem))
        pl.when((j >= 0) & (j < TAIL_COL // 512))(lambda: project(j))

    cols = pl.ds(TAIL_COL, BLOCK_COLS)
    o = attention_out(cols)
    for k, (_, (tile, ntiles)) in enumerate(TAIL):
        wo = wo_buf.at[pl.ds(2 * tile, 2 * ntiles), :, cols]
        wait_for(wo, tail_sems.at[k])
        lo, n = 128 * tile, 128 * ntiles
        y = y_ref[:, lo:lo + n] + lax.dot_general(
            o, wo[...].reshape(n, BLOCK_COLS), NT_DIMS, preferred_element_type=f32)
        lane = lo + lax.broadcasted_iota(jnp.int32, (1, n), 1)
        out_ref[0, :, lo:lo + n] = jnp.where(lane < D, y[0:1], y[4:5]).astype(out_ref.dtype)


def _kernel(*refs):
    dma = pltpu.SemaphoreType.DMA
    pl.run_scoped(functools.partial(_body, *refs),
                  dma(()), dma(()), dma(()), dma((LAG + 1,)), dma((len(TAIL),)))


@jax.jit
def pallas_concat_heads__gqa_block_cached__sliding_block_cached__decode_kernel(
    A_x: jax.Array,
    A_k_cache: jax.Array,
    A_v_cache: jax.Array,
    A_wq: jax.Array,
    A_wo: jax.Array,
    B_x: jax.Array,
    B_k_cache: jax.Array,
    B_v_cache: jax.Array,
    B_wq: jax.Array,
    B_wo: jax.Array,
):
    f32, bf16 = jnp.float32, jnp.bfloat16

    def views(x, k, v, wq, wo):
        cache, weight = (HKV, 2, SK // 2, DH), (NSLAB, SLAB, HQ * DH)
        return (x, k.reshape(cache), v.reshape(cache), wq.reshape(weight), wo.T.reshape(weight))

    return pl.pallas_call(
        _kernel,
        out_shape=jax.ShapeDtypeStruct((1, 1, 2 * D), bf16),
        in_specs=[pl.BlockSpec(memory_space=pltpu.HBM)] * 10,
        scratch_shapes=[
            pltpu.VMEM((2, 1, D), bf16),
            pltpu.VMEM((2 * NSLAB, SLAB, HQ * DH), bf16),
            pltpu.VMEM((2 * NSLAB, SLAB, HQ * DH), bf16),
            pltpu.VMEM((GROUPS, 2, HEADS, KEYS // PIECE, PIECE, DH), bf16),
            pltpu.VMEM((8, DH), f32),
            pltpu.VMEM((8, DH), f32),
            pltpu.VMEM((8, DH), f32),
            pltpu.VMEM((8, DH), f32),
            pltpu.VMEM((2, 8, HQ * DH), f32),
            pltpu.VMEM((8, 2 * D), f32),
        ],
        compiler_params=pltpu.CompilerParams(vmem_limit_bytes=108 * 2**20),
    )(*views(A_x, A_k_cache, A_v_cache, A_wq, A_wo), *views(B_x, B_k_cache, B_v_cache, B_wq, B_wo))
```
